```python
import jax
import jax.numpy as jnp

def _softmax(x, axis=-1):
    return jax.nn.softmax(x, axis=axis)
def _gelu(x):
    return jax.nn.gelu(x, approximate=True)
def _silu(x):
    return jax.nn.silu(x)
def _sigmoid(x):
    return jax.nn.sigmoid(x)
def _layernorm(x, axis=-1, eps=1e-5):
    m = jnp.mean(x, axis=axis, keepdims=True)
    v = jnp.var(x, axis=axis, keepdims=True)
    return (x - m) / jnp.sqrt(v + eps)
def _scatter_add(tgt, idx, src, axis=0):
    return tgt.at[idx].add(src)
def _segment_sum(src, seg, n):
    return jax.ops.segment_sum(src, seg, n)
class _Rng:
    def __init__(self, key):
        self._k = key
    def _next(self):
        self._k, sub = jax.random.split(self._k)
        return sub
    def normal(self, shape):
        return jax.random.normal(self._next(), shape, dtype=jnp.bfloat16)
    def randint(self, lo, hi, shape):
        return jax.random.randint(self._next(), shape, lo, hi, dtype=jnp.int32)
    def uniform(self, shape, lo=0.0, hi=1.0):
        return jax.random.uniform(self._next(), shape, jnp.bfloat16, lo, hi)
    def permutation(self, n):
        return jax.random.permutation(self._next(), n)


kernel_name = 'sequential_preLN__sliding_block_cached__moe_arch_mod__decode'

def setup_inputs():
    _rng = _Rng(jax.random.key(int.from_bytes(__import__("os").urandom(4), "little")))
    _w = (lambda a: (lambda t: t.astype(jnp.bfloat16) if jnp.issubdtype(t.dtype, jnp.floating) else t)(jnp.asarray(a)))
    def _A_setup():
        B, Sq, D = 1, 1, 640
        Hq, Hkv, Sk, Dh = 32, 32, 32768, 192
        assert Hq % Hkv == 0, (Hq, Hkv)
        return {
            "x": _w((lambda *s: _rng.normal(s) * 0.05)(B, Sq, D)),
            "k_cache": _w((lambda *s: _rng.normal(s) * 0.05)(B, Hkv, Sk, Dh)),
            "v_cache": _w((lambda *s: _rng.normal(s) * 0.05)(B, Hkv, Sk, Dh)),
            "wq": _w((lambda *s: _rng.normal(s) * 0.05)(D, Hq * Dh) * (D ** -0.5)),
            "wo": _w((lambda *s: _rng.normal(s) * 0.05)(Hq * Dh, D) * ((Hq * Dh) ** -0.5)),
        }
    _A_in = _A_setup()

    def _B_setup():
        B, S, D, F, C = 1, 1, 640, 1536, 1
        return {
            "x": _w((lambda *s: _rng.normal(s) * 0.05)(B, S, D)),
            "w_r": _w((lambda *s: _rng.normal(s) * 0.05)(D)),
            "w_gate": _w((lambda *s: _rng.normal(s) * 0.05)(D, F)),
            "w_up": _w((lambda *s: _rng.normal(s) * 0.05)(D, F)),
            "w_down": _w((lambda *s: _rng.normal(s) * 0.05)(F, D)),
        }
    _B_in = _B_setup()

    return {
        "A_x": _A_in["x"],
        "A_k_cache": _A_in["k_cache"],
        "A_v_cache": _A_in["v_cache"],
        "A_wq": _A_in["wq"],
        "A_wo": _A_in["wo"],
        "B_x": _B_in["x"],
        "B_w_r": _B_in["w_r"],
        "B_w_gate": _B_in["w_gate"],
        "B_w_up": _B_in["w_up"],
        "B_w_down": _B_in["w_down"],
    }

def reference(A_x, A_k_cache, A_v_cache, A_wq, A_wo, B_x, B_w_r, B_w_gate, B_w_up, B_w_down):
    def _A_ref(x, k_cache, v_cache, wq, wo):
        B, Sq, D = x.shape
        Hq, Dh = 32, 192
        Hkv, Sk = k_cache.shape[1], k_cache.shape[2]
        W = min(4096, max(256, Sk // 4))
        rep = Hq // Hkv
        q = (lambda x, *d: x.transpose(*d))((x @ wq).reshape(B, Sq, Hq, Dh), 0, 2, 1, 3)
        k = jnp.repeat(k_cache[:, :, Sk - W:, :], rep, axis=1)
        v = jnp.repeat(v_cache[:, :, Sk - W:, :], rep, axis=1)
        scores = jnp.einsum("bhqd,bhkd->bhqk", q, k) * (Dh ** -0.5)
        p = _softmax(scores, axis=-1)
        o = jnp.einsum("bhqk,bhkd->bhqd", p, v)
        return (lambda x, *d: x.transpose(*d))(o, 0, 2, 1, 3).reshape(B, Sq, Hq * Dh) @ wo

    def _B_ref(x, w_r, w_gate, w_up, w_down):
        B, S, D = x.shape
        C = 1
        r = x @ w_r
        idx = jnp.argsort(-r, axis=-1)[:, :C]
        idx_e = jnp.repeat(idx.reshape(B, C, 1), D, axis=2)
        x_sel = jnp.take_along_axis(x, idx_e, axis=1)
        g = _silu(x_sel @ w_gate)
        u = x_sel @ w_up
        y = (g * u) @ w_down
        r_sel = _sigmoid(jnp.take_along_axis(r, idx, axis=1))
        y = y * r_sel.reshape(B, C, 1)
        b_off = (jnp.arange(B) * S).reshape(B, 1)
        flat_idx = (idx + b_off).reshape(B * C)
        zero = (x * 0.0).reshape(B * S, D)
        upd = _scatter_add(zero, flat_idx, y.reshape(B * C, D), axis=0)
        return x + upd.reshape(B, S, D)

    x = A_x
    h = x + _A_ref(_layernorm(x, axis=-1), A_k_cache, A_v_cache, A_wq, A_wo)
    h2 = h + _B_ref(_layernorm(h, axis=-1), B_w_r, B_w_gate, B_w_up, B_w_down)
    return h2
```

```python
import functools

import jax
import jax.numpy as jnp
from jax import lax
import jax.experimental.pallas as pl
import jax.experimental.pallas.tpu as pltpu

EPS = 1e-5
SKEW = 24
KV_ROWS, KV_COLS = 32, 512
WQ_COLS = 2048
WO_ROWS = 24
WD_ROWS = 16
CHUNKS = 4
WD_PARTS = ((0, 256, 768, 1024), (256, 768), (1024, 1408), (1408, 1536))


def _layernorm(x):
    m = jnp.mean(x, axis=-1, keepdims=True)
    d = x - m
    v = jnp.mean(d * d, axis=-1, keepdims=True)
    return d / jnp.sqrt(v + EPS)


def _div3(i):
    return (i * 21846) >> 16


def _zip_runs(t0, t1):
    out, lists = [], [[list(x) for x in t0], [list(x) for x in t1]]
    while any(lists):
        n = min(x[0][2] for x in lists if x)
        out.append((n, *(tuple(x[0][:2]) if x else None for x in lists)))
        for x in lists:
            if x:
                x[0][1] += n
                x[0][2] -= n
                if not x[0][2]:
                    x.pop(0)
    return out


def _split(runs, m):
    return [(min(m, n - s), a and (a[0], a[1] + s), b and (b[0], b[1] + s))
            for n, a, b in runs for s in range(0, n, m)]


def _run(n, a, b):
    def step(i, carry):
        if b:
            b[0](b[1] + i, 1)
        if a:
            a[0](a[1] + i, 0)
        return carry
    lax.fori_loop(0, n, step, 0)


def _weave(runs, work):
    n = len(work)
    for j, w in enumerate(work):
        for r in runs[j * len(runs) // n:(j + 1) * len(runs) // n]:
            _run(*r)
        w()


def _done(dst, sem):
    pltpu.make_async_copy(dst, dst, sem).wait()


def _kernel(x_hbm, k_hbm, v_hbm, wq_hbm, wo_hbm, wr_hbm, wg_hbm, wu_hbm, wd_hbm, o_ref,
            x_s, wr_s, k_s, v_s, wq_s, wo_s, wg_s, wu_s, wd_s, s_s, p_s, acc_s,
            sem_k, sem_v, sem_w, sem_d, *, head_dim):
    f32, bf16 = jnp.float32, jnp.bfloat16
    R, W = k_s.shape
    Sk = k_hbm.shape[1]
    D, F = wg_s.shape
    Dh = head_dim
    P = 2 * Dh
    NP = R // P

    def copy(src, dst, sem, queue, r, nr, c, nc, off=0):
        rows = pl.ds(pl.multiple_of(r, 8), nr)
        if isinstance(c, int):
            cols, src_cols = pl.ds(c, nc), pl.ds(c + off, nc)
        else:
            cols, src_cols = pl.ds(pl.multiple_of(c, 128), nc), pl.ds(pl.multiple_of(c + off, 128), nc)
        pltpu.make_async_copy(src.at[rows, src_cols], dst.at[rows, cols], sem).start(priority=queue)

    def wq_piece(i, t):
        j = i >> 2
        a = _div3(j)
        copy(wq_hbm, wq_s, sem_w.at[0], t, (((i & 3) + 4 * t) * (D // 64) + a) * 8, 8,
             (j - 3 * a) * WQ_COLS, WQ_COLS)

    def wo_piece(i, t):
        r = (((i & 3) + 4 * t) * (R // WO_ROWS // 8) + (i >> 2)) * WO_ROWS
        copy(wo_hbm, wo_s, sem_w.at[1], t, r, WO_ROWS, 0, D)

    def cache_piece(src, dst, sem, head):
        def piece(i, t):
            c = _div3(i)
            r = head * Dh + t * (Dh // 2) + (i - 3 * c) * KV_ROWS
            copy(src, dst, sem, t, r, KV_ROWS, c * KV_COLS, KV_COLS, Sk - W)
        return piece

    def gu_piece(i, t):
        r = ((i & 3) * (D // 32) + (i >> 2)) * 8
        copy((wg_hbm, wu_hbm)[t], (wg_s, wu_s)[t], sem_w.at[2], t, r, 8, 0, F)

    def wd_pieces(t):
        lo_t, hi_t = t * (F // 2), (t + 1) * (F // 2)
        spans = sorted((lo, hi, c) for c, b in enumerate(WD_PARTS)
                       for lo, hi in zip(b[0::2], b[1::2]) if lo_t <= lo < hi_t)
        return [(lambda i, t, c=c: copy(wd_hbm, wd_s, sem_d.at[c], t, i * WD_ROWS, WD_ROWS, 0, D),
                 lo // WD_ROWS, (hi - lo) // WD_ROWS) for lo, hi, c in spans]

    def pair_pieces(p):
        return [cache_piece(src, dst, sem.at[p & 1], 2 * p + h)
                for src, dst, sem in ((k_hbm, k_s, sem_k), (v_hbm, v_s, sem_v)) for h in range(2)]

    NQ = (D // 8) * (R // WQ_COLS) // 2
    NO = R // WO_ROWS // 2
    NG = D // 8
    NS = (W // KV_COLS) * (Dh // 2 // KV_ROWS)
    assert R == 3 * WQ_COLS and Dh == 6 * KV_ROWS and NS == SKEW

    row = lax.broadcasted_iota(jnp.int32, (8, P), 0)
    col = lax.broadcasted_iota(jnp.int32, (8, P), 1)
    own = row == jnp.where(col < Dh, 0, 1)
    scale = Dh ** -0.5
    CW = W // CHUNKS

    def attend(p, xn):
        st = {}
        rows = pl.ds(p * P if isinstance(p, int) else pl.multiple_of(p * P, P), P)

        def q_proj():
            q = jnp.dot(xn, wq_s[:, rows], preferred_element_type=f32)
            st["q"] = jnp.where(own, q, 0.0).astype(bf16)
            _done(k_s.at[rows], sem_k.at[p & 1])

        def qk(c):
            cols = slice(c * CW, (c + 1) * CW)
            s_s[:, cols] = jnp.dot(st["q"], k_s[rows, cols], preferred_element_type=f32) * scale

        def softmax():
            s = s_s[...]
            e = jnp.exp(s - jnp.max(s, axis=-1, keepdims=True))
            st["inv"] = 1.0 / jnp.sum(e, axis=-1, keepdims=True)
            p_s[...] = e
            _done(v_s.at[rows], sem_v.at[p & 1])

        def pv(c):
            cols = slice(c * CW, (c + 1) * CW)
            o = lax.dot_general(p_s[:, cols].astype(bf16), v_s[rows, cols], (((1,), (1,)), ((), ())),
                                preferred_element_type=f32)
            st["o"] = o if c == 0 else st["o"] + o

        def out_proj():
            o = jnp.where(own, st["o"] * st["inv"], 0.0).astype(bf16)
            acc_s[...] += jnp.dot(o, wo_s[rows, :], preferred_element_type=f32)

        return ([q_proj] + [functools.partial(qk, c) for c in range(CHUNKS)],
                [softmax] + [functools.partial(pv, c) for c in range(CHUNKS)] + [out_proj])

    x_cp = pltpu.make_async_copy(x_hbm, x_s, sem_w.at[3])
    wr_cp = pltpu.make_async_copy(wr_hbm, wr_s, sem_w.at[4])
    _run(SKEW, None, (wq_piece, 0))
    for r in _zip_runs([(wq_piece, 0, NQ)], [(wq_piece, SKEW, NQ - SKEW), (wo_piece, 0, SKEW)]):
        _run(*r)
    wr_cp.start(priority=1)
    x_cp.start(priority=0)
    first = pair_pieces(0)
    for r in _zip_runs([(wo_piece, 0, NO)], [(wo_piece, SKEW, NO - SKEW), (first[0], 0, SKEW)]):
        _run(*r)
    x_cp.wait()
    x = x_s[0].astype(f32)
    xn = jnp.broadcast_to(_layernorm(x), (8, D)).astype(bf16)
    acc_s[...] = jnp.zeros_like(acc_s)
    for a, b in zip(first, first[1:] + [pair_pieces(1)[0]]):
        _run(NS, (a, 0), (b, 0))
    _done(wq_s, sem_w.at[0])
    _done(wo_s, sem_w.at[1])

    def pair(p, ahead):
        cur = pair_pieces(p)
        runs = [(NS, (a, 0), (b, 0)) for a, b in zip(cur, cur[1:] + [ahead])]
        scores, values = attend(p - 1, xn)
        _weave(_split(runs[:2], NS // 4), scores)
        _weave(_split(runs[2:], NS // 4), values)

    def body(p, carry):
        pair(p, pair_pieces(p + 1)[0])
        return carry

    lax.fori_loop(1, NP - 1, body, 0)
    pair(NP - 1, gu_piece)

    scores, values = attend(NP - 1, xn)
    runs = _zip_runs([(gu_piece, 0, NG)] + wd_pieces(0), [(gu_piece, SKEW, NG - SKEW)] + wd_pieces(1))
    head = _split(runs[:1], 4)
    _weave(head[:len(head) // 2], scores)
    _weave(head[len(head) // 2:], values)

    h = x + jnp.sum(acc_s[...], axis=0, keepdims=True)
    hn = _layernorm(h)
    wr_cp.wait()
    wr = wr_s[...].astype(f32).reshape(1, D)
    gate = jax.nn.sigmoid(jnp.sum(hn * wr, axis=-1, keepdims=True))
    hb = jnp.broadcast_to(hn, (8, D)).astype(bf16)
    for r in runs[1:]:
        _run(*r)
    _done(wg_s, sem_w.at[2])
    _done(wu_s, sem_w.at[2])
    g = jnp.dot(hb, wg_s[...], preferred_element_type=f32)
    u = jnp.dot(hb, wu_s[...], preferred_element_type=f32)
    gu = (g * jax.nn.sigmoid(g) * u).astype(bf16)
    y = jnp.zeros((8, D), f32)
    for c, b in enumerate(WD_PARTS):
        spans = list(zip(b[0::2], b[1::2]))
        for lo, hi in spans:
            _done(wd_s.at[pl.ds(lo, hi - lo)], sem_d.at[c])
        for lo, hi in spans:
            y = y + jnp.dot(gu[:, lo:hi], wd_s[lo:hi, :], preferred_element_type=f32)
    o_ref[0] = (h + (hn + y[:1] * gate)).astype(o_ref.dtype)


@jax.jit
def pallas_sequential_preLN__sliding_block_cached__moe_arch_mod__decode_kernel(
    A_x: jax.Array,
    A_k_cache: jax.Array,
    A_v_cache: jax.Array,
    A_wq: jax.Array,
    A_wo: jax.Array,
    B_x: jax.Array,
    B_w_r: jax.Array,
    B_w_gate: jax.Array,
    B_w_up: jax.Array,
    B_w_down: jax.Array,
):
    del B_x
    _, H, Sk, Dh = A_k_cache.shape
    D = A_x.shape[-1]
    W = min(4096, max(256, Sk // 4))
    kt = jnp.transpose(A_k_cache, (0, 1, 3, 2)).reshape(H * Dh, Sk)
    vt = jnp.transpose(A_v_cache, (0, 1, 3, 2)).reshape(H * Dh, Sk)
    like = lambda a: pltpu.VMEM(a.shape, a.dtype)
    sems = lambda n: pltpu.SemaphoreType.DMA((n,))
    return pl.pallas_call(
        functools.partial(_kernel, head_dim=Dh),
        out_shape=jax.ShapeDtypeStruct(A_x.shape, A_x.dtype),
        in_specs=[pl.BlockSpec(memory_space=pl.ANY)] * 9,
        scratch_shapes=[
            like(A_x), like(B_w_r),
            pltpu.VMEM((H * Dh, W), A_k_cache.dtype), pltpu.VMEM((H * Dh, W), A_v_cache.dtype),
            like(A_wq), like(A_wo), like(B_w_gate), like(B_w_up), like(B_w_down),
            pltpu.VMEM((8, W), jnp.float32), pltpu.VMEM((8, W), jnp.float32),
            pltpu.VMEM((8, D), jnp.float32),
            sems(2), sems(2), sems(5), sems(len(WD_PARTS)),
        ],
        compiler_params=pltpu.CompilerParams(
            vmem_limit_bytes=126 * 2**20, disable_bounds_checks=True, disable_semaphore_checks=True),
    )(A_x, kt, vt, A_wq, A_wo, B_w_r, B_w_gate, B_w_up, B_w_down)
```

```python
import functools

import jax
import jax.numpy as jnp
from jax import lax
import jax.experimental.pallas as pl
import jax.experimental.pallas.tpu as pltpu

EPS = 1e-5
SKEW = 27
FIRST = 4
KV_ROWS, KV_COLS = 32, 512
RANGE_ROWS = 2048
RANGES_PER_COPY, ROWS_PER_COPY = 3, 32
CHUNKS = 4
WD_COPIES = (((0, 768, 32),), ((768, 1488, 16), (1488, 1536, 8)))
WD_MXU = (((0, 512), (768, 1024)), ((512, 768), (1024, 1152)))
WD_VPU = (((1152, 1280),), ((1280, 1408),), ((1408, 1504),), ((1504, 1536),))


def _layernorm(x):
    m = jnp.mean(x, axis=-1, keepdims=True)
    d = x - m
    v = jnp.mean(d * d, axis=-1, keepdims=True)
    return d / jnp.sqrt(v + EPS)


def _column(row):
    return jnp.broadcast_to(row, (128, 128)).T


def _div(i, m):
    if m & (m - 1) == 0:
        return i >> (m.bit_length() - 1)
    return (i * (-(-(1 << 16) // m))) >> 16


def _aligned(v, m):
    return v if isinstance(v, int) else pl.multiple_of(v, m)


def _drop(segments, n):
    head, rest = [], []
    for piece, first, count in segments:
        k = min(n, count)
        n -= k
        if k:
            head.append((piece, first, k))
        if count - k:
            rest.append((piece, first + k, count - k))
    return head, rest


def _zip_runs(queue0, queue1):
    out, lists = [], [[list(s) for s in queue0], [list(s) for s in queue1]]
    while any(lists):
        n = min(x[0][2] for x in lists if x)
        out.append((n, *(tuple(x[0][:2]) if x else None for x in lists)))
        for x in lists:
            if x:
                x[0][1] += n
                x[0][2] -= n
                if not x[0][2]:
                    x.pop(0)
    return out


def _cut(runs, bounds):
    out, cur, pos, bounds = [], [], 0, list(bounds)
    for n, a, b in runs:
        s = 0
        while s < n:
            k = min(n - s, bounds[0] - pos) if bounds else n - s
            cur.append((k, a and (a[0], a[1] + s), b and (b[0], b[1] + s)))
            s += k
            pos += k
            if bounds and bounds[0] == pos:
                out.append(cur)
                cur = []
                bounds.pop(0)
    return out + [cur]


def _issue(runs):
    for n, a, b in runs:
        def step(i, carry, a=a, b=b):
            if b:
                b[0](b[1] + i, 1)
            if a:
                a[0](a[1] + i, 0)
            return carry
        if n == 1:
            step(0, 0)
        else:
            lax.fori_loop(0, n, step, 0)


def _weave(runs, work):
    n = sum(r[0] for r in runs)
    for group, w in zip(_cut(runs, [(j + 1) * n // len(work) for j in range(len(work) - 1)]), work):
        _issue(group)
        w()


def _done(dst, sem):
    pltpu.make_async_copy(dst, dst, sem).wait()


def _kernel(x_hbm, k_hbm, v_hbm, wq_hbm, wo_hbm, wr_hbm, wg_hbm, wu_hbm, wd_hbm, o_ref,
            x_s, wr_s, k_s, v_s, wq_s, wo_s, wg_s, wu_s, wd_s,
            xc_s, q_s, s_s, p_s, acc_s, gc_s,
            sem_k, sem_v, sem_w, sem_d, *, head_dim):
    f32, bf16 = jnp.float32, jnp.bfloat16
    R, W = k_s.shape
    Sk = k_hbm.shape[1]
    D, F = wg_s.shape
    Dh = head_dim
    P = 2 * Dh
    NP = R // P

    def copy(src, dst, sem, queue, r, nr, c, nc, src_offset=0):
        rows = pl.ds(_aligned(r, 8), nr)
        pltpu.make_async_copy(src.at[rows, pl.ds(_aligned(c + src_offset, 128), nc)],
                              dst.at[rows, pl.ds(_aligned(c, 128), nc)], sem).start(priority=queue)

    def qo_piece(i, t):
        m = wq_hbm.shape[0] // RANGES_PER_COPY
        b = _div(i, m)
        idx = (pl.ds((i - m * b) * RANGES_PER_COPY, RANGES_PER_COPY),
               pl.ds(_aligned(b * ROWS_PER_COPY, ROWS_PER_COPY), ROWS_PER_COPY))
        src, dst = ((wq_hbm, wq_s), (wo_hbm, wo_s))[t]
        pltpu.make_async_copy(src.at[idx], dst.at[idx], sem_w.at[t]).start(priority=t)

    col_blocks = W // KV_COLS
    row_blocks = Dh // 2 // KV_ROWS
    NS = 2 * col_blocks * row_blocks

    def pair_segments(p):
        def window(src, dst, sem):
            def piece(i, t):
                c = _div(i, row_blocks)
                h = _div(c, col_blocks)
                r = p * P + h * Dh + t * (Dh // 2) + (i - row_blocks * c) * KV_ROWS
                copy(src, dst, sem, t, r, KV_ROWS, (c - col_blocks * h) * KV_COLS, KV_COLS, Sk - W)
            return piece
        return [(window(k_hbm, k_s, sem_k.at[p & 1]), 0, NS), (window(v_hbm, v_s, sem_v.at[p & 1]), 0, NS)]

    def gu_piece(i, t):
        r = ((i & 3) * (D // 32) + (i >> 2)) * 8
        copy((wg_hbm, wu_hbm)[t], (wg_s, wu_s)[t], sem_w.at[2], t, r, 8, 0, F)

    def wd_segments(t):
        out = []
        for first, last, n in WD_COPIES[t]:
            spans = sorted((max(lo, first), min(hi, last), c) for c, group in enumerate(WD_MXU + WD_VPU)
                           for lo, hi in group if lo < last and hi > first)
            for lo, hi, c in spans:
                assert (hi - lo) % n == 0
                out.append((lambda i, t, lo=lo, n=n, c=c: copy(wd_hbm, wd_s, sem_d.at[c], t, lo + i * n, n, 0, D),
                            0, (hi - lo) // n))
        return out

    x_cp = pltpu.make_async_copy(x_hbm, x_s, sem_w.at[3])
    wr_cp = pltpu.make_async_copy(wr_hbm, wr_s, sem_w.at[4])
    vectors = (lambda i, t: (x_cp, wr_cp)[t].start(priority=t), 0, 1)

    def tiles(ref, n):
        per_range = RANGE_ROWS // 128
        a = _div(n, per_range)
        return ref[a, pl.ds(_aligned((n - a * per_range) * 128, 128), 128), :].astype(f32)

    def q_steps():
        st, per_row, unroll = {}, R // 2048, 4

        def half(c, h):
            def rows(i, acc):
                for u in range(unroll):
                    r = i * unroll + u
                    w = tiles(wq_s, r * per_row + c)
                    xc = xc_s[pl.ds(pl.multiple_of(r * 8, 8), 8), :]
                    acc = tuple(acc[j] + xc * w[j * 8:(j + 1) * 8] for j in range(16))
                return acc
            n = D // 16 // unroll
            start = st[c] if h else tuple(jnp.zeros((8, 128), f32) for _ in range(16))
            st[c] = lax.fori_loop(h * n, (h + 1) * n, rows, start)
            if h:
                q = jnp.sum(jnp.concatenate(st[c], axis=1), axis=0, keepdims=True)
                q_s[:, c * 2048:(c + 1) * 2048] = jnp.broadcast_to(q, (8, 2048))

        return [functools.partial(half, c, h) for c in range(per_row) for h in range(2)]

    def attend(p):
        st = {}
        rows = pl.ds(_aligned(p * P, P), P)
        scale = Dh ** -0.5
        cw = W // CHUNKS

        def own():
            return (lax.broadcasted_iota(jnp.int32, (8, P), 0)
                    == jnp.where(lax.broadcasted_iota(jnp.int32, (8, P), 1) < Dh, 0, 1))

        def queries():
            st["q"] = jnp.where(own(), q_s[:, rows], 0.0).astype(bf16)
            _done(k_s.at[rows], sem_k.at[p & 1])

        def qk(c):
            cols = slice(c * cw, (c + 1) * cw)
            s_s[:, cols] = jnp.dot(st["q"], k_s[rows, cols], preferred_element_type=f32) * scale

        def softmax():
            s = s_s[...]
            e = jnp.exp(s - jnp.max(s, axis=-1, keepdims=True))
            st["inv"] = 1.0 / jnp.sum(e, axis=-1, keepdims=True)
            p_s[...] = e
            _done(v_s.at[rows], sem_v.at[p & 1])

        def pv(c):
            cols = slice(c * cw, (c + 1) * cw)
            o = lax.dot_general(p_s[:, cols].astype(bf16), v_s[rows, cols], (((1,), (1,)), ((), ())),
                                preferred_element_type=f32)
            st["o"] = o if c == 0 else st["o"] + o

        def out_proj():
            o = jnp.sum(jnp.where(own(), st["o"] * st["inv"], 0.0), axis=0, keepdims=True)
            nj = D // 128
            acc = [acc_s[:, j * 128:(j + 1) * 128] for j in range(nj)]
            for b in range(P // 128):
                oc = _column(o[:, b * 128:(b + 1) * 128])
                for n in range(nj):
                    w = tiles(wo_s, (p * (P // 128) + b) * nj + n)
                    for a in range(16):
                        i, j = divmod(n * 16 + a, nj)
                        acc[j] = acc[j] + oc[i * 8:(i + 1) * 8] * w[a * 8:(a + 1) * 8]
            acc_s[...] = jnp.concatenate(acc, axis=1)

        return ([queries] + [functools.partial(qk, c) for c in range(CHUNKS)],
                [softmax] + [functools.partial(pv, c) for c in range(CHUNKS)] + [out_proj])

    NQ = wq_hbm.shape[0] // RANGES_PER_COPY * (RANGE_ROWS // ROWS_PER_COPY)
    head = [(qo_piece, 0, NQ // 2), vectors, (qo_piece, NQ // 2, NQ - NQ // 2)] + pair_segments(0)
    lead, rest = _drop(head, FIRST + SKEW)
    for i in range(FIRST):
        qo_piece(i, 1)
        qo_piece(i, 0)
    _issue(_zip_runs([], _drop(lead, FIRST)[1]))
    runs = _zip_runs(_drop(head, FIRST)[1], rest + _drop(pair_segments(1), SKEW)[0])
    early, late = _cut(runs, [sum(r[0] for r in runs) - 2 * NS + 32])
    _issue(early)
    x_cp.wait()
    x = x_s[0].astype(f32)
    xn = _layernorm(x)
    for b in range(D // 128):
        xc_s[b * 128:(b + 1) * 128, :] = _column(xn[:, b * 128:(b + 1) * 128])
    acc_s[...] = jnp.zeros_like(acc_s)
    _done(wq_s, sem_w.at[0])
    _done(wo_s, sem_w.at[1])
    _weave(late, q_steps())

    def pair(p, ahead):
        cur = pair_segments(p)
        first, second = _cut(_zip_runs(cur, _drop(cur, SKEW)[1] + _drop(ahead, SKEW)[0]), [NS])
        scores, values = attend(p - 1)
        _weave(first, scores)
        _weave(second, values)

    def body(p, carry):
        pair(p, pair_segments(p + 1))
        return carry

    lax.fori_loop(1, NP - 1, body, 0)
    tail = [[(gu_piece, 0, D // 8)] + wd_segments(t) for t in range(2)]
    pair(NP - 1, tail[1])

    first, second, third = _cut(_zip_runs(tail[0], _drop(tail[1], SKEW)[1]), [26, 52])
    scores, values = attend(NP - 1)
    _weave(first, scores)
    _weave(second, values)

    h = x + jnp.sum(acc_s[...], axis=0, keepdims=True)
    hn = _layernorm(h)
    wr_cp.wait()
    wr = wr_s[...].astype(f32).reshape(1, D)
    gate = jax.nn.sigmoid(jnp.sum(hn * wr, axis=-1, keepdims=True))
    hb = jnp.broadcast_to(hn, (8, D)).astype(bf16)
    _issue(third)
    _done(wg_s, sem_w.at[2])
    _done(wu_s, sem_w.at[2])
    g = jnp.dot(hb, wg_s[...], preferred_element_type=f32)
    u = jnp.dot(hb, wu_s[...], preferred_element_type=f32)
    gu = (g * jax.nn.sigmoid(g) * u).astype(bf16)
    v0 = F - gc_s.shape[0]
    for r in range(v0, F, 128):
        gc_s[r - v0:r - v0 + 128, :] = _column(gu[:1, r:r + 128].astype(f32) * gate)

    y = jnp.zeros((8, D), f32)
    for c, group in enumerate(WD_MXU):
        for lo, hi in group:
            _done(wd_s.at[pl.ds(lo, hi - lo)], sem_d.at[c])
        for lo, hi in group:
            y = y + jnp.dot(gu[:, lo:hi], wd_s[lo:hi, :], preferred_element_type=f32)
    out = jnp.where(lax.broadcasted_iota(jnp.int32, (8, D), 0) == 0, h + (hn + y[:1] * gate), 0.0)
    for c, group in enumerate(WD_VPU):
        for lo, hi in group:
            _done(wd_s.at[pl.ds(lo, hi - lo)], sem_d.at[len(WD_MXU) + c])
        for lo, hi in group:
            for r in range(lo, hi, 8):
                gc = gc_s[r - v0:r - v0 + 8, :]
                out = out + wd_s[r:r + 8, :].astype(f32) * jnp.concatenate([gc] * (D // 128), axis=1)
    o_ref[0] = jnp.sum(out, axis=0, keepdims=True).astype(o_ref.dtype)


def _as_tiles(w):
    m, n = w.shape
    return w.reshape(m // 8, 8, n // 128, 128).transpose(0, 2, 1, 3).reshape(-1, RANGE_ROWS, 128)


@jax.jit
def pallas_sequential_preLN__sliding_block_cached__moe_arch_mod__decode_kernel(
    A_x: jax.Array,
    A_k_cache: jax.Array,
    A_v_cache: jax.Array,
    A_wq: jax.Array,
    A_wo: jax.Array,
    B_x: jax.Array,
    B_w_r: jax.Array,
    B_w_gate: jax.Array,
    B_w_up: jax.Array,
    B_w_down: jax.Array,
):
    del B_x
    _, H, Sk, Dh = A_k_cache.shape
    D = A_x.shape[-1]
    F = B_w_down.shape[0]
    W = min(4096, max(256, Sk // 4))
    kt = jnp.transpose(A_k_cache, (0, 1, 3, 2)).reshape(H * Dh, Sk)
    vt = jnp.transpose(A_v_cache, (0, 1, 3, 2)).reshape(H * Dh, Sk)
    wq, wo = _as_tiles(A_wq), _as_tiles(A_wo)
    like = lambda a: pltpu.VMEM(a.shape, a.dtype)
    f32 = lambda *shape: pltpu.VMEM(shape, jnp.float32)
    sems = lambda n: pltpu.SemaphoreType.DMA((n,))
    return pl.pallas_call(
        functools.partial(_kernel, head_dim=Dh),
        out_shape=jax.ShapeDtypeStruct(A_x.shape, A_x.dtype),
        in_specs=[pl.BlockSpec(memory_space=pl.ANY)] * 9,
        scratch_shapes=[
            like(A_x), like(B_w_r),
            pltpu.VMEM((H * Dh, W), A_k_cache.dtype), pltpu.VMEM((H * Dh, W), A_v_cache.dtype),
            like(wq), like(wo), like(B_w_gate), like(B_w_up), like(B_w_down),
            f32(D, 128), f32(8, H * Dh), f32(8, W), f32(8, W), f32(8, D), f32(F - WD_VPU[0][0][0], 128),
            sems(2), sems(2), sems(5), sems(len(WD_MXU) + len(WD_VPU)),
        ],
        compiler_params=pltpu.CompilerParams(
            vmem_limit_bytes=126 * 2**20, disable_bounds_checks=True, disable_semaphore_checks=True),
    )(A_x, kt, vt, wq, wo, B_w_r, B_w_gate, B_w_up, B_w_down)
```

```python
import functools

import jax
import jax.numpy as jnp
from jax import lax
import jax.experimental.pallas as pl
import jax.experimental.pallas.tpu as pltpu

EPS = 1e-5
SKEW = 27
FIRST = 3
KV_ROWS, KV_COLS = 24, 512
RANGE_ROWS = 2048
RANGES_PER_COPY, ROWS_PER_COPY = 3, 32
CHUNKS = 4
WD_COPIES = (((0, 768, 32),), ((768, 1488, 16), (1488, 1536, 8)))
WD_MXU = (((0, 512), (768, 1024)), ((512, 768), (1024, 1152)))
WD_VPU = ((1152, 1280), (1280, 1408), (1408, 1488), (1488, 1520), (1520, 1536))
WD_SPANS = tuple(span for group in WD_MXU for span in group) + WD_VPU


def _layernorm(x):
    m = jnp.mean(x, axis=-1, keepdims=True)
    d = x - m
    v = jnp.mean(d * d, axis=-1, keepdims=True)
    return d / jnp.sqrt(v + EPS)


def _column(row):
    return jnp.broadcast_to(row, (128, 128)).T


def _div(i, m):
    if m & (m - 1) == 0:
        return i >> (m.bit_length() - 1)
    return (i * (-(-(1 << 16) // m))) >> 16


def _aligned(v, m):
    return v if isinstance(v, int) else pl.multiple_of(v, m)


def _drop(segments, n):
    head, rest = [], []
    for piece, first, count in segments:
        k = min(n, count)
        n -= k
        if k:
            head.append((piece, first, k))
        if count - k:
            rest.append((piece, first + k, count - k))
    return head, rest


def _zip_runs(queue0, queue1):
    out, lists = [], [[list(s) for s in queue0], [list(s) for s in queue1]]
    while any(lists):
        n = min(x[0][2] for x in lists if x)
        out.append((n, *(tuple(x[0][:2]) if x else None for x in lists)))
        for x in lists:
            if x:
                x[0][1] += n
                x[0][2] -= n
                if not x[0][2]:
                    x.pop(0)
    return out


def _cut(runs, bounds):
    out, cur, pos, bounds = [], [], 0, list(bounds)
    for n, a, b in runs:
        s = 0
        while s < n:
            k = min(n - s, bounds[0] - pos) if bounds else n - s
            cur.append((k, a and (a[0], a[1] + s), b and (b[0], b[1] + s)))
            s += k
            pos += k
            if bounds and bounds[0] == pos:
                out.append(cur)
                cur = []
                bounds.pop(0)
    return out + [cur]


def _issue(runs):
    for n, a, b in runs:
        def step(i, carry, a=a, b=b):
            if b:
                b[0](b[1] + i, 1)
            if a:
                a[0](a[1] + i, 0)
            return carry
        if n == 1:
            step(0, 0)
        else:
            lax.fori_loop(0, n, step, 0)


def _weave(runs, work):
    n = sum(r[0] for r in runs)
    for group, w in zip(_cut(runs, [(j + 1) * n // len(work) for j in range(len(work) - 1)]), work):
        _issue(group)
        w()


def _done(dst, sem):
    pltpu.make_async_copy(dst, dst, sem).wait()


def _kernel(x_hbm, k_hbm, v_hbm, wq_hbm, wo_hbm, wr_hbm, wg_hbm, wu_hbm, wd_hbm, o_ref,
            x_s, wr_s, k_s, v_s, wq_s, wo_s, wg_s, wu_s, wd_s,
            xc_s, q_s, s_s, p_s, acc_s, gc_s,
            sem_k, sem_v, sem_w, sem_d, *, head_dim):
    f32, bf16 = jnp.float32, jnp.bfloat16
    R, W = k_s.shape
    Sk = k_hbm.shape[1]
    D, F = wg_s.shape
    Dh = head_dim
    P = 2 * Dh
    NP = R // P
    assert R % P == 0 and P % 128 == 0 and R % 2048 == 0 and D % 128 == 0 and D % 64 == 0
    assert W % KV_COLS == 0 and Dh % (2 * KV_ROWS) == 0 and wq_hbm.shape[0] % RANGES_PER_COPY == 0
    assert sorted(WD_SPANS)[-1][1] == F and sum(hi - lo for lo, hi in WD_SPANS) == F

    def copy(src, dst, sem, queue, r, nr, c, nc, src_offset=0):
        rows = pl.ds(_aligned(r, 8), nr)
        pltpu.make_async_copy(src.at[rows, pl.ds(_aligned(c + src_offset, 128), nc)],
                              dst.at[rows, pl.ds(_aligned(c, 128), nc)], sem).start(priority=queue)

    def qo_piece(i, t):
        m = wq_hbm.shape[0] // RANGES_PER_COPY
        b = _div(i, m)
        idx = (pl.ds((i - m * b) * RANGES_PER_COPY, RANGES_PER_COPY),
               pl.ds(_aligned(b * ROWS_PER_COPY, ROWS_PER_COPY), ROWS_PER_COPY))
        src, dst = ((wq_hbm, wq_s), (wo_hbm, wo_s))[t]
        pltpu.make_async_copy(src.at[idx], dst.at[idx], sem_w.at[t]).start(priority=t)

    col_blocks = W // KV_COLS
    row_blocks = Dh // 2 // KV_ROWS
    NS = 2 * col_blocks * row_blocks

    def pair_segments(p):
        def window(src, dst, sem):
            def piece(i, t):
                c = _div(i, row_blocks)
                h = _div(c, col_blocks)
                r = p * P + h * Dh + t * (Dh // 2) + (i - row_blocks * c) * KV_ROWS
                copy(src, dst, sem, t, r, KV_ROWS, (c - col_blocks * h) * KV_COLS, KV_COLS, Sk - W)
            return piece
        return [(window(k_hbm, k_s, sem_k.at[p & 1]), 0, NS), (window(v_hbm, v_s, sem_v.at[p & 1]), 0, NS)]

    def gu_piece(i, t):
        r = ((i & 3) * (D // 32) + (i >> 2)) * 8
        copy((wg_hbm, wu_hbm)[t], (wg_s, wu_s)[t], sem_w.at[2 + t], t, r, 8, 0, F)

    def wd_segments(t):
        out = []
        for first, last, n in WD_COPIES[t]:
            spans = sorted((max(lo, first), min(hi, last), c) for c, (lo, hi) in enumerate(WD_SPANS)
                           if lo < last and hi > first)
            for lo, hi, c in spans:
                assert (hi - lo) % n == 0
                out.append((lambda i, t, lo=lo, n=n, c=c: copy(wd_hbm, wd_s, sem_d.at[c], t, lo + i * n, n, 0, D),
                            0, (hi - lo) // n))
        return out

    x_cp = pltpu.make_async_copy(x_hbm, x_s, sem_w.at[4])
    wr_cp = pltpu.make_async_copy(wr_hbm, wr_s, sem_w.at[5])
    vectors = (lambda i, t: (x_cp, wr_cp)[t].start(priority=t), 0, 1)

    def tiles(ref, n):
        per_range = RANGE_ROWS // 128
        a = _div(n, per_range)
        return ref[a, pl.ds(_aligned((n - a * per_range) * 128, 128), 128), :].astype(f32)

    def q_steps():
        st, per_row, unroll = {}, R // 2048, 4

        def half(c, h):
            def rows(i, acc):
                for u in range(unroll):
                    r = i * unroll + u
                    w = tiles(wq_s, r * per_row + c)
                    xc = xc_s[pl.ds(pl.multiple_of(r * 8, 8), 8), :]
                    acc = tuple(acc[j] + xc * w[j * 8:(j + 1) * 8] for j in range(16))
                return acc
            n = D // 16 // unroll
            start = st[c] if h else tuple(jnp.zeros((8, 128), f32) for _ in range(16))
            st[c] = lax.fori_loop(h * n, (h + 1) * n, rows, start)
            if h:
                q = jnp.sum(jnp.concatenate(st[c], axis=1), axis=0, keepdims=True)
                q_s[:, c * 2048:(c + 1) * 2048] = jnp.broadcast_to(q, (8, 2048))

        return [functools.partial(half, c, h) for c in range(per_row) for h in range(2)]

    def attend(p):
        st = {}
        rows = pl.ds(_aligned(p * P, P), P)
        scale = Dh ** -0.5
        cw = W // CHUNKS

        def own():
            return (lax.broadcasted_iota(jnp.int32, (8, P), 0)
                    == jnp.where(lax.broadcasted_iota(jnp.int32, (8, P), 1) < Dh, 0, 1))

        def queries():
            st["q"] = jnp.where(own(), q_s[:, rows], 0.0).astype(bf16)
            _done(k_s.at[rows], sem_k.at[p & 1])

        def qk(c):
            cols = slice(c * cw, (c + 1) * cw)
            s_s[:, cols] = jnp.dot(st["q"], k_s[rows, cols], preferred_element_type=f32) * scale

        def softmax():
            s = s_s[...]
            e = jnp.exp(s - jnp.max(s, axis=-1, keepdims=True))
            st["inv"] = 1.0 / jnp.sum(e, axis=-1, keepdims=True)
            p_s[...] = e
            _done(v_s.at[rows], sem_v.at[p & 1])

        def pv(c):
            cols = slice(c * cw, (c + 1) * cw)
            o = lax.dot_general(p_s[:, cols].astype(bf16), v_s[rows, cols], (((1,), (1,)), ((), ())),
                                preferred_element_type=f32)
            st["o"] = o if c == 0 else st["o"] + o

        def out_proj():
            o = jnp.sum(jnp.where(own(), st["o"] * st["inv"], 0.0), axis=0, keepdims=True)
            nj = D // 128
            acc = [acc_s[:, j * 128:(j + 1) * 128] for j in range(nj)]
            for b in range(P // 128):
                oc = _column(o[:, b * 128:(b + 1) * 128])
                for n in range(nj):
                    w = tiles(wo_s, (p * (P // 128) + b) * nj + n)
                    for a in range(16):
                        i, j = divmod(n * 16 + a, nj)
                        acc[j] = acc[j] + oc[i * 8:(i + 1) * 8] * w[a * 8:(a + 1) * 8]
            acc_s[...] = jnp.concatenate(acc, axis=1)

        return ([queries] + [functools.partial(qk, c) for c in range(CHUNKS)],
                [softmax] + [functools.partial(pv, c) for c in range(CHUNKS)] + [out_proj])

    NQ = wq_hbm.shape[0] // RANGES_PER_COPY * (RANGE_ROWS // ROWS_PER_COPY)
    head = [(qo_piece, 0, NQ // 2), vectors, (qo_piece, NQ // 2, NQ - NQ // 2)] + pair_segments(0)
    for i in range(FIRST + SKEW):
        qo_piece(i, 1)
        if i < FIRST:
            qo_piece(i, 0)
    runs = _zip_runs(_drop(head, FIRST)[1], _drop(head, FIRST + SKEW)[1] + _drop(pair_segments(1), SKEW)[0])
    early, late = _cut(runs, [sum(r[0] for r in runs) - 2 * NS + 40])
    _issue(early)
    x_cp.wait()
    x = x_s[0].astype(f32)
    xn = _layernorm(x)
    for b in range(D // 128):
        xc_s[b * 128:(b + 1) * 128, :] = _column(xn[:, b * 128:(b + 1) * 128])
    acc_s[...] = jnp.zeros_like(acc_s)
    _done(wq_s, sem_w.at[0])
    _done(wo_s, sem_w.at[1])
    _weave(late, q_steps())

    def pair(p, ahead):
        cur = pair_segments(p)
        first, second = _cut(_zip_runs(cur, _drop(cur, SKEW)[1] + _drop(ahead, SKEW)[0]), [NS])
        scores, values = attend(p - 1)
        _weave(first, scores)
        _weave(second, values)

    def body(p, carry):
        pair(p, pair_segments(p + 1))
        return carry

    lax.fori_loop(1, NP - 1, body, 0)
    tail = [[(gu_piece, 0, D // 8)] + wd_segments(t) for t in range(2)]
    pair(NP - 1, tail[1])

    first, second, third = _cut(_zip_runs(tail[0], _drop(tail[1], SKEW)[1]), [26, 52])
    scores, values = attend(NP - 1)
    _weave(first, scores)
    _weave(second, values)

    h = x + jnp.sum(acc_s[...], axis=0, keepdims=True)
    hn = _layernorm(h)
    wr_cp.wait()
    wr = wr_s[...].astype(f32).reshape(1, D)
    gate = jax.nn.sigmoid(jnp.sum(hn * wr, axis=-1, keepdims=True))
    hb = jnp.broadcast_to(hn, (8, D)).astype(bf16)
    _issue(third)
    _done(wg_s, sem_w.at[2])
    _done(wu_s, sem_w.at[3])
    g = jnp.dot(hb, wg_s[...], preferred_element_type=f32)
    u = jnp.dot(hb, wu_s[...], preferred_element_type=f32)
    gu = (g * jax.nn.sigmoid(g) * u).astype(bf16)
    v0 = F - gc_s.shape[0]
    for r in range(v0, F, 128):
        gc_s[r - v0:r - v0 + 128, :] = _column(gu[:1, r:r + 128].astype(f32) * gate)

    def wd_done(lo, hi):
        _done(wd_s.at[pl.ds(lo, hi - lo)], sem_d.at[WD_SPANS.index((lo, hi))])

    y = jnp.zeros((8, D), f32)
    for group in WD_MXU:
        for lo, hi in group:
            wd_done(lo, hi)
        for lo, hi in group:
            y = y + jnp.dot(gu[:, lo:hi], wd_s[lo:hi, :], preferred_element_type=f32)
    out = jnp.where(lax.broadcasted_iota(jnp.int32, (8, D), 0) == 0, h + (hn + y[:1] * gate), 0.0)
    for lo, hi in WD_VPU:
        wd_done(lo, hi)
        for r in range(lo, hi, 8):
            gc = gc_s[r - v0:r - v0 + 8, :]
            out = out + wd_s[r:r + 8, :].astype(f32) * jnp.concatenate([gc] * (D // 128), axis=1)
    o_ref[0] = jnp.sum(out, axis=0, keepdims=True).astype(o_ref.dtype)


def _as_tiles(w):
    m, n = w.shape
    return w.reshape(m // 8, 8, n // 128, 128).transpose(0, 2, 1, 3).reshape(-1, RANGE_ROWS, 128)


@jax.jit
def pallas_sequential_preLN__sliding_block_cached__moe_arch_mod__decode_kernel(
    A_x: jax.Array,
    A_k_cache: jax.Array,
    A_v_cache: jax.Array,
    A_wq: jax.Array,
    A_wo: jax.Array,
    B_x: jax.Array,
    B_w_r: jax.Array,
    B_w_gate: jax.Array,
    B_w_up: jax.Array,
    B_w_down: jax.Array,
):
    del B_x
    _, H, Sk, Dh = A_k_cache.shape
    D = A_x.shape[-1]
    F = B_w_down.shape[0]
    W = min(4096, max(256, Sk // 4))
    kt = jnp.transpose(A_k_cache, (0, 1, 3, 2)).reshape(H * Dh, Sk)
    vt = jnp.transpose(A_v_cache, (0, 1, 3, 2)).reshape(H * Dh, Sk)
    wq, wo = _as_tiles(A_wq), _as_tiles(A_wo)
    like = lambda a: pltpu.VMEM(a.shape, a.dtype)
    f32 = lambda *shape: pltpu.VMEM(shape, jnp.float32)
    sems = lambda n: pltpu.SemaphoreType.DMA((n,))
    return pl.pallas_call(
        functools.partial(_kernel, head_dim=Dh),
        out_shape=jax.ShapeDtypeStruct(A_x.shape, A_x.dtype),
        in_specs=[pl.BlockSpec(memory_space=pl.ANY)] * 9,
        scratch_shapes=[
            like(A_x), like(B_w_r),
            pltpu.VMEM((H * Dh, W), A_k_cache.dtype), pltpu.VMEM((H * Dh, W), A_v_cache.dtype),
            like(wq), like(wo), like(B_w_gate), like(B_w_up), like(B_w_down),
            f32(D, 128), f32(8, H * Dh), f32(8, W), f32(8, W), f32(8, D), f32(F - WD_VPU[0][0], 128),
            sems(2), sems(2), sems(6), sems(len(WD_SPANS)),
        ],
        compiler_params=pltpu.CompilerParams(
            vmem_limit_bytes=126 * 2**20, disable_bounds_checks=True, disable_semaphore_checks=True),
    )(A_x, kt, vt, wq, wo, B_w_r, B_w_gate, B_w_up, B_w_down)
```
